```python
import jax
import jax.numpy as jnp

def _softmax(x, axis=-1):
    return jax.nn.softmax(x, axis=axis)
def _gelu(x):
    return jax.nn.gelu(x, approximate=True)
def _silu(x):
    return jax.nn.silu(x)
def _sigmoid(x):
    return jax.nn.sigmoid(x)
def _layernorm(x, axis=-1, eps=1e-5):
    m = jnp.mean(x, axis=axis, keepdims=True)
    v = jnp.var(x, axis=axis, keepdims=True)
    return (x - m) / jnp.sqrt(v + eps)
def _scatter_add(tgt, idx, src, axis=0):
    return tgt.at[idx].add(src)
def _segment_sum(src, seg, n):
    return jax.ops.segment_sum(src, seg, n)
class _Rng:
    def __init__(self, key):
        self._k = key
    def _next(self):
        self._k, sub = jax.random.split(self._k)
        return sub
    def normal(self, shape):
        return jax.random.normal(self._next(), shape, dtype=jnp.bfloat16)
    def randint(self, lo, hi, shape):
        return jax.random.randint(self._next(), shape, lo, hi, dtype=jnp.int32)
    def uniform(self, shape, lo=0.0, hi=1.0):
        return jax.random.uniform(self._next(), shape, jnp.bfloat16, lo, hi)
    def permutation(self, n):
        return jax.random.permutation(self._next(), n)


kernel_name = 'gated_mix__mha_block_cached__compressed_kv_cla__decode'

def setup_inputs():
    _rng = _Rng(jax.random.key(int.from_bytes(__import__("os").urandom(4), "little")))
    _w = (lambda a: (lambda t: t.astype(jnp.bfloat16) if jnp.issubdtype(t.dtype, jnp.floating) else t)(jnp.asarray(a)))
    def _A_setup():
        B, Sq, D = 2, 1, 512
        H, Sk, Dh = 32, 8192, 128
        return {
            "x": _w((lambda *s: _rng.normal(s) * 0.05)(B, Sq, D)),
            "k_cache": _w((lambda *s: _rng.normal(s) * 0.05)(B, H, Sk, Dh)),
            "v_cache": _w((lambda *s: _rng.normal(s) * 0.05)(B, H, Sk, Dh)),
            "wq": _w((lambda *s: _rng.normal(s) * 0.05)(D, H * Dh) * (D ** -0.5)),
            "wo": _w((lambda *s: _rng.normal(s) * 0.05)(H * Dh, D) * ((H * Dh) ** -0.5)),
        }
    _A_in = _A_setup()

    def _B_setup():
        B, H, Sq, Sk, D, M = 2, 32, 1, 8192, 128, 512
        Dc = 4 * D
        return {
            "x": _w((lambda *s: _rng.normal(s) * 0.05)(B, Sq, M)),
            "c_kv": _w((lambda *s: _rng.normal(s) * 0.05)(B, Sk, Dc)),
            "w_q": _w((lambda *s: _rng.normal(s) * 0.05)(M, H, D) * (M ** -0.5)),
            "w_uk": _w((lambda *s: _rng.normal(s) * 0.05)(Dc, H, D) * (Dc ** -0.5)),
            "w_uv": _w((lambda *s: _rng.normal(s) * 0.05)(Dc, H, D) * (Dc ** -0.5)),
            "w_o": _w((lambda *s: _rng.normal(s) * 0.05)(H, D, M) * ((H * D) ** -0.5)),
        }
    _B_in = _B_setup()

    return {
        "A_x": _A_in["x"],
        "A_k_cache": _A_in["k_cache"],
        "A_v_cache": _A_in["v_cache"],
        "A_wq": _A_in["wq"],
        "A_wo": _A_in["wo"],
        "B_x": _B_in["x"],
        "B_c_kv": _B_in["c_kv"],
        "B_w_q": _B_in["w_q"],
        "B_w_uk": _B_in["w_uk"],
        "B_w_uv": _B_in["w_uv"],
        "B_w_o": _B_in["w_o"],
        "gate_w": _w((lambda *s: _rng.normal(s) * 0.05)(512)),
    }

def reference(A_x, A_k_cache, A_v_cache, A_wq, A_wo, B_x, B_c_kv, B_w_q, B_w_uk, B_w_uv, B_w_o, gate_w):
    def _A_ref(x, k_cache, v_cache, wq, wo):
        B, Sq, D = x.shape
        H, Dh = 32, 128
        q = (lambda x, *d: x.transpose(*d))((x @ wq).reshape(B, Sq, H, Dh), 0, 2, 1, 3)
        scores = jnp.einsum("bhqd,bhkd->bhqk", q, k_cache) * (Dh ** -0.5)
        p = _softmax(scores, axis=-1)
        o = jnp.einsum("bhqk,bhkd->bhqd", p, v_cache)
        return (lambda x, *d: x.transpose(*d))(o, 0, 2, 1, 3).reshape(B, Sq, H * Dh) @ wo

    def _B_ref(x, c_kv, w_q, w_uk, w_uv, w_o):
        B, Sq, M = x.shape[0], x.shape[1], x.shape[2]
        Sk = c_kv.shape[1]
        H, D = w_q.shape[1], w_q.shape[2]
        q = jnp.einsum("bqm,mhd->bhqd", x, w_q)
        k = jnp.einsum("bkc,chd->bhkd", c_kv, w_uk)
        v = jnp.einsum("bkc,chd->bhkd", c_kv, w_uv)
        scores = jnp.einsum("bhqd,bhkd->bhqk", q, k) * (D ** -0.5)
        off = Sk - Sq
        qi = jnp.arange(Sq)[:, None]
        kj = jnp.arange(Sk)[None, :]
        cmask = kj <= (qi + off)
        scores = jnp.where(cmask[None, None], scores, -1e9)
        p = _softmax(scores, axis=-1)
        ctx = jnp.einsum("bhqk,bhkd->bhqd", p, v)
        return jnp.einsum("bhqd,hdm->bqm", ctx, w_o)

    x = A_x
    g = _sigmoid((x * gate_w).sum(-1, keepdims=True))
    a = _A_ref(x, A_k_cache, A_v_cache, A_wq, A_wo)
    b = _B_ref(x, B_c_kv, B_w_q, B_w_uk, B_w_uv, B_w_o)
    return g * a + (1 - g) * b
```

```python
import jax
import jax.numpy as jnp
from jax import lax
import jax.experimental.pallas as pl
import jax.experimental.pallas.tpu as pltpu

_B, _H, _SK, _DH, _D = 2, 32, 8192, 128, 512
_RING = 16
_CH = 2048
_NT = (((1,), (1,)), ((), ()))
_F32 = jnp.float32
_BF16 = jnp.bfloat16


def _dot(a, b):
    return jnp.dot(a, b, preferred_element_type=_F32)


def _dot_nt(a, b):
    return lax.dot_general(a, b, _NT, preferred_element_type=_F32)


def _kernel(x_ref, gw_ref, k_hbm, v_hbm, wqa_hbm, woa_hbm, c_hbm, wqb_hbm, wuk_hbm,
            wuv_hbm, wob_hbm, o_ref,
            ring, wqa, woa, cbuf, wqb, wuk, wuv, wob, u32, qa_ref, qabs_ref, s_ref,
            ctx_ref, outb_ref, ring_sem, w_sem):
    scale = _DH ** -0.5

    def kv_copy(c, slot):
        h = c // 4
        b = (c // 2) % 2
        return h, b

    def kv_start_static(c):
        h, b, isv = c // 4, (c // 2) % 2, c % 2
        src = v_hbm if isv else k_hbm
        pltpu.make_async_copy(src.at[b, h], ring.at[c % _RING], ring_sem.at[c % _RING]).start()

    def kv_start(c, b, isv):
        h = c // 4
        slot = c % _RING
        src = v_hbm if isv else k_hbm
        pltpu.make_async_copy(src.at[b, h], ring.at[slot], ring_sem.at[slot]).start()

    def kv_wait(slot):
        pltpu.make_async_copy(k_hbm.at[0, 0], ring.at[slot], ring_sem.at[slot]).wait()

    cp_wqa = pltpu.make_async_copy(wqa_hbm, wqa, w_sem.at[0])
    cp_woa = pltpu.make_async_copy(woa_hbm, woa, w_sem.at[1])
    cp_wqb = pltpu.make_async_copy(wqb_hbm, wqb, w_sem.at[2])
    cp_wuk = pltpu.make_async_copy(wuk_hbm, wuk, w_sem.at[3])
    cp_wuv = pltpu.make_async_copy(wuv_hbm, wuv, w_sem.at[4])
    cp_wob = pltpu.make_async_copy(wob_hbm, wob, w_sem.at[5])
    cp_c = [pltpu.make_async_copy(c_hbm.at[b], cbuf.at[b], w_sem.at[6 + b]) for b in range(_B)]

    cp_wqa.start()
    kv_start_static(0)
    kv_start_static(1)
    cp_woa.start()
    for c in range(2, _RING):
        kv_start_static(c)

    row8 = lax.broadcasted_iota(jnp.int32, (8, _D), 0)
    x0 = jnp.broadcast_to(x_ref[0].astype(_F32), (8, _D))
    x1 = jnp.broadcast_to(x_ref[1].astype(_F32), (8, _D))
    x8 = jnp.where(row8 == 0, x0, jnp.where(row8 == 1, x1, 0.0))
    gw = gw_ref[...].reshape(1, _D).astype(_F32)
    g = jax.nn.sigmoid(jnp.sum(x8 * gw, axis=1, keepdims=True))

    cp_wqa.wait()
    x8b = x8.astype(_BF16)
    for h in range(_H):
        qa_ref[h] = _dot(x8b, wqa[:, h * _DH:(h + 1) * _DH])

    row16 = lax.broadcasted_iota(jnp.int32, (16, _D), 0) % 8
    row16h = lax.broadcasted_iota(jnp.int32, (16, _DH), 0) % 8

    def to_u32(w):
        def body(i, _):
            v = w[pl.ds(pl.multiple_of(i * 1024, 1024), 1024), :]
            u32[pl.ds(pl.multiple_of(i * 512, 512), 512), :] = pltpu.bitcast(v, jnp.uint32)
            return _
        lax.fori_loop(0, 16384 // 1024, body, 0)

    def head_pair(j):
        u = u32[pl.ds(j, _D, stride=16), :]
        lo = pltpu.bitcast(u << 16, _F32).astype(_BF16)
        hi = pltpu.bitcast(u & jnp.uint32(0xFFFF0000), _F32).astype(_BF16)
        return lo, hi

    def b_stage_q():
        x16 = jnp.concatenate([x0, x1], axis=0)
        cp_wqb.wait()
        to_u32(wqb)
        qs = []
        for gi in range(4):
            acc = jnp.zeros((16, _DH), _F32)
            for jj in range(4):
                ws = head_pair(4 * gi + jj)
                for hh in range(2):
                    r = 2 * jj + hh
                    lhs = jnp.where(row16 == r, x16, 0.0).astype(_BF16)
                    acc = acc + _dot(lhs, ws[hh])
            qs.append(acc)
        cp_wuk.wait()
        to_u32(wuk)
        for gi in range(4):
            acc = jnp.zeros((16, _D), _F32)
            for jj in range(4):
                ws = head_pair(4 * gi + jj)
                for hh in range(2):
                    r = 2 * jj + hh
                    lhs = jnp.where(row16h == r, qs[gi], 0.0).astype(_BF16)
                    acc = acc + _dot_nt(lhs, ws[hh])
            qabs_ref[0, gi * 8:(gi + 1) * 8, :] = acc[0:8]
            qabs_ref[1, gi * 8:(gi + 1) * 8, :] = acc[8:16]

    def b_stage_attn(b):
        cp_c[b].wait()
        qb = qabs_ref[b].astype(_BF16)
        nch = _SK // _CH

        def p1(i, mx):
            off = pl.multiple_of(i * _CH, _CH)
            s = _dot_nt(qb, cbuf[b, pl.ds(off, _CH), :]) * scale
            s_ref[i] = s
            for t in range(_CH // 128):
                mx = jnp.maximum(mx, s[:, t * 128:(t + 1) * 128])
            return mx
        mx = lax.fori_loop(0, nch, p1, jnp.full((_H, 128), -jnp.inf, _F32))
        m = jnp.max(mx, axis=1, keepdims=True)

        def p2(i, carry):
            l, acc = carry
            off = pl.multiple_of(i * _CH, _CH)
            p = jnp.exp(s_ref[i] - m)
            for t in range(_CH // 128):
                l = l + p[:, t * 128:(t + 1) * 128]
            acc = acc + _dot(p.astype(_BF16), cbuf[b, pl.ds(off, _CH), :])
            return l, acc
        l, acc = lax.fori_loop(0, nch, p2, (jnp.zeros((_H, 128), _F32),
                                            jnp.zeros((_H, _D), _F32)))
        ctx_ref[b] = acc / jnp.sum(l, axis=1, keepdims=True)

    def b_stage_out():
        cp_wuv.wait()
        to_u32(wuv)
        cp_wob.wait()
        out16 = jnp.zeros((16, _D), _F32)
        for gi in range(4):
            cg = jnp.concatenate([ctx_ref[0, gi * 8:(gi + 1) * 8, :],
                                  ctx_ref[1, gi * 8:(gi + 1) * 8, :]], axis=0)
            acc = jnp.zeros((16, _DH), _F32)
            for jj in range(4):
                ws = head_pair(4 * gi + jj)
                for hh in range(2):
                    r = 2 * jj + hh
                    lhs = jnp.where(row16 == r, cg, 0.0).astype(_BF16)
                    acc = acc + _dot(lhs, ws[hh])
            for r in range(8):
                h = gi * 8 + r
                lhs = jnp.where(row16h == r, acc, 0.0).astype(_BF16)
                out16 = out16 + _dot(lhs, wob[h * _DH:(h + 1) * _DH, :])
        s0 = jnp.sum(out16[0:8], axis=0, keepdims=True)
        s1 = jnp.sum(out16[8:16], axis=0, keepdims=True)
        outb_ref[...] = jnp.where(row8 == 0, s0, jnp.where(row8 == 1, s1, 0.0))

    row8h = lax.broadcasted_iota(jnp.int32, (8, _DH), 0)
    nchunks = 4 * _H

    def a_head(h, outa):
        @pl.when(h == 1)
        def _():
            cp_wqb.start()
            cp_wuk.start()

        @pl.when(h == 2)
        def _():
            cp_c[0].start()

        @pl.when(h == 4)
        def _():
            cp_c[1].start()

        @pl.when(h == 6)
        def _():
            cp_wuv.start()
            cp_wob.start()

        @pl.when(h == 7)
        def _():
            b_stage_q()

        @pl.when(h == 9)
        def _():
            b_stage_attn(0)

        @pl.when(h == 11)
        def _():
            b_stage_attn(1)

        @pl.when(h == 13)
        def _():
            b_stage_out()

        @pl.when(h == 0)
        def _():
            cp_woa.wait()

        q8 = qa_ref[h].astype(_BF16)
        on = []
        for b in range(_B):
            ck = 4 * h + 2 * b
            ks = ck % _RING
            vs = (ck + 1) % _RING
            kv_wait(ks)
            s = _dot_nt(q8, ring[ks]) * scale

            @pl.when(ck + _RING < nchunks)
            def _():
                kv_start(ck + _RING, b, 0)
            m = jnp.max(s, axis=1, keepdims=True)
            p = jnp.exp(s - m)
            l = jnp.sum(p, axis=1, keepdims=True)
            kv_wait(vs)
            o = _dot(p.astype(_BF16), ring[vs])

            @pl.when(ck + 1 + _RING < nchunks)
            def _():
                kv_start(ck + 1 + _RING, b, 1)
            on.append(o / l)
        lhs = jnp.where(row8h == 0, on[0], jnp.where(row8h == 1, on[1], 0.0)).astype(_BF16)
        hoff = pl.multiple_of(h * _DH, _DH)
        return outa + _dot(lhs, woa[pl.ds(hoff, _DH), :])

    outa = lax.fori_loop(0, _H, a_head, jnp.zeros((8, _D), _F32))

    res = (g * outa + (1.0 - g) * outb_ref[...]).astype(_BF16)
    o_ref[0] = res[0:1]
    o_ref[1] = res[1:2]


@jax.jit
def pallas_gated_mix__mha_block_cached__compressed_kv_cla__decode_kernel(
    A_x: jax.Array,
    A_k_cache: jax.Array,
    A_v_cache: jax.Array,
    A_wq: jax.Array,
    A_wo: jax.Array,
    B_x: jax.Array,
    B_c_kv: jax.Array,
    B_w_q: jax.Array,
    B_w_uk: jax.Array,
    B_w_uv: jax.Array,
    B_w_o: jax.Array,
    gate_w: jax.Array,
):
    del B_x
    any_spec = pl.BlockSpec(memory_space=pl.ANY)
    vmem_spec = pl.BlockSpec(memory_space=pltpu.VMEM)
    hd = _H * _DH
    scratch = [
        pltpu.VMEM((_RING, _SK, _DH), _BF16),
        pltpu.VMEM((_D, hd), _BF16),
        pltpu.VMEM((hd, _D), _BF16),
        pltpu.VMEM((_B, _SK, _D), _BF16),
        pltpu.VMEM((_D * _H, _DH), _BF16),
        pltpu.VMEM((_D * _H, _DH), _BF16),
        pltpu.VMEM((_D * _H, _DH), _BF16),
        pltpu.VMEM((hd, _D), _BF16),
        pltpu.VMEM((_D * _H // 2, _DH), jnp.uint32),
        pltpu.VMEM((_H, 8, _DH), _F32),
        pltpu.VMEM((_B, _H, _D), _F32),
        pltpu.VMEM((_SK // _CH, _H, _CH), _F32),
        pltpu.VMEM((_B, _H, _D), _F32),
        pltpu.VMEM((8, _D), _F32),
        pltpu.SemaphoreType.DMA((_RING,)),
        pltpu.SemaphoreType.DMA((8,)),
    ]
    return pl.pallas_call(
        _kernel,
        out_shape=jax.ShapeDtypeStruct((_B, 1, _D), _BF16),
        in_specs=[vmem_spec, vmem_spec] + [any_spec] * 9,
        out_specs=vmem_spec,
        scratch_shapes=scratch,
        compiler_params=pltpu.CompilerParams(vmem_limit_bytes=110 * 1024 * 1024),
    )(A_x, gate_w, A_k_cache, A_v_cache, A_wq, A_wo, B_c_kv,
      B_w_q.reshape(_D * _H, _DH), B_w_uk.reshape(_D * _H, _DH),
      B_w_uv.reshape(_D * _H, _DH), B_w_o.reshape(hd, _D))
```

```python
import jax
import jax.numpy as jnp
import numpy as np
from jax import lax
import jax.experimental.pallas as pl
import jax.experimental.pallas.tpu as pltpu

_B, _H, _SK, _DH, _D = 2, 32, 8192, 128, 512
_NT = (((1,), (1,)), ((), ()))
_F32 = jnp.float32
_BF16 = jnp.bfloat16
_HI16 = np.uint32(0xFFFF0000)

_LA = 2
_NSTEP = 4
_KV = (4, (32, 64))
_W3 = (4, (32, 64))
_WO = (2, (16,))
_CK = (2, (16, 32))
_WQA = (16, (2560, 1536))
_NP = 8
_T0 = 4
_CH = 2048
_SUB = 512


def _dot(a, b):
    return jnp.dot(a, b, preferred_element_type=_F32)


def _dot_nt(a, b):
    return lax.dot_general(a, b, _NT, preferred_element_type=_F32)


def _plan(total, sizes):
    out, o = [], 0
    while o < total:
        w = min(sizes[len(out) % len(sizes)], total - o)
        out.append((o, w, len(out) % 2))
        o += w
    return out


def _split(n, parts):
    return [(n * i) // parts for i in range(parts + 1)]


def _chunks(lst, parts):
    c = _split(len(lst), parts)
    return [lst[c[i]:c[i + 1]] for i in range(parts)]


def _kernel(x_hbm, gw_hbm, k_hbm, v_hbm, wqa_hbm, woa_hbm, c_hbm, wqb_hbm, wuk_hbm,
            wuv_hbm, wob_hbm, o_ref,
            x_ref, gw_ref, kbuf, vbuf, wqa, woa, cbuf, wqb, wuk, wuv, wob, u32,
            qa_ref, q_ref, qabs_ref, s_ref, mx_ref, l_ref, acc_ref, ctx_ref, outb_ref,
            k_sem, v_sem, w_sem):
    scale = _DH ** -0.5
    nst = _B * _H
    g_kv, r_kv = _KV[0], _SK // _KV[0]
    r_w3, r_wo, r_ck = _D * _H // _W3[0], _H * _DH // _WO[0], _SK // 2 // _CK[0]
    kv_plan, w3_plan = _plan(r_kv, _KV[1]), _plan(r_w3, _W3[1])
    wo_plan, ck_plan = _plan(r_wo, _WO[1]), _plan(r_ck, _CK[1])

    def descs3(src, dst, plan, sem):
        return [(src.at[:, pl.ds(o, w), :], dst.at[:, pl.ds(o, w), :], pr, sem)
                for (o, w, pr) in plan]

    def issue(descs, cond=None):
        def go():
            for (src, dst, pr, sem) in descs:
                pltpu.make_async_copy(src, dst, sem).start(priority=pr)
        if descs and cond is None:
            go()
        elif descs:
            pl.when(cond)(go)

    def wait_all(dst, sem):
        pltpu.make_async_copy(dst, dst, sem).wait()

    def run(gen, n, carry):
        cut = _split(len(carry), n)
        for i in range(n):
            issue(carry[cut[i]:cut[i + 1]])
            next(gen)
        for _ in gen:
            pass

    def kv_descs(t, b):
        h, slot = t // 2, t % _NSTEP
        hs = pl.ds(h * g_kv, g_kv)
        return (descs3(k_hbm.at[b, hs], kbuf.at[slot], kv_plan, k_sem.at[slot])
                + descs3(v_hbm.at[b, hs], vbuf.at[slot], kv_plan, v_sem.at[slot]))

    d_wqa = []
    for r0 in range(0, _D, _WQA[0]):
        c0 = 0
        for nc in _WQA[1]:
            idx = (pl.ds(r0, _WQA[0]), pl.ds(c0, nc))
            d_wqa.append((wqa_hbm.at[idx], wqa.at[idx], len(d_wqa) % 2, w_sem.at[0]))
            c0 += nc
    d_woa = descs3(woa_hbm, woa, wo_plan, w_sem.at[1])
    d_wqb = descs3(wqb_hbm, wqb, w3_plan, w_sem.at[2])
    d_wuk = descs3(wuk_hbm, wuk, w3_plan, w_sem.at[3])
    d_wuv = descs3(wuv_hbm, wuv, w3_plan, w_sem.at[4])
    d_wob = descs3(wob_hbm, wob, wo_plan, w_sem.at[5])
    d_c = [descs3(c_hbm.at[b, hf], cbuf.at[b, hf], ck_plan, w_sem.at[6 + 2 * b + hf])
           for b in range(_B) for hf in range(2)]

    cp_x = pltpu.make_async_copy(x_hbm, x_ref, w_sem.at[10])
    cp_g = pltpu.make_async_copy(gw_hbm, gw_ref, w_sem.at[11])
    issue(d_wqa[:4])
    cp_x.start()
    cp_g.start()
    issue(d_wqa[4:])
    issue(kv_descs(0, 0))
    u32[pl.ds(_D * _H // 2, 16), :] = jnp.zeros((16, _DH), jnp.uint32)
    cp_x.wait()
    cp_g.wait()

    row8 = lax.broadcasted_iota(jnp.int32, (8, _D), 0)
    xf = x_ref[...].astype(_F32)
    x0 = jnp.broadcast_to(xf[0:1], (8, _D))
    x1 = jnp.broadcast_to(xf[1:2], (8, _D))
    x8 = jnp.where(row8 == 0, x0, jnp.where(row8 == 1, x1, 0.0))
    gw = gw_ref[...].reshape(1, _D).astype(_F32)
    g = jax.nn.sigmoid(jnp.sum(x8 * gw, axis=1, keepdims=True))

    def qa_gen():
        wait_all(wqa, w_sem.at[0])
        x8b = x8.astype(_BF16)
        for h in range(_H):
            qa_ref[h] = _dot(x8b, wqa[:, h * _DH:(h + 1) * _DH])
            yield
    carry0 = d_woa
    for t in range(_LA - 1, 0, -1):
        carry0 = kv_descs(t, t % 2) + carry0
    run(qa_gen(), _H, carry0)

    row16 = lax.broadcasted_iota(jnp.int32, (16, _D), 0) % 8
    row16h = lax.broadcasted_iota(jnp.int32, (16, _DH), 0) % 8

    def to_u32(w, sem):
        def gen():
            wait_all(w, sem)
            n = r_w3 // 1024
            for i in range(16):
                v = w[i // n, pl.ds((i % n) * 1024, 1024), :]
                u32[pl.ds(i * 512, 512), :] = pltpu.bitcast(v, jnp.uint32)
                yield
        return gen, 16

    def head_pair(j):
        u = u32[pl.ds(j, _D, stride=16), :]
        lo = pltpu.bitcast(u << 16, _F32).astype(_BF16)
        hi = pltpu.bitcast(u & _HI16, _F32).astype(_BF16)
        return lo, hi

    def q_piece(gis):
        def gen():
            x16 = jnp.concatenate([x0, x1], axis=0)
            for gi in gis:
                acc = jnp.zeros((16, _DH), _F32)
                for jj in range(4):
                    ws = head_pair(4 * gi + jj)
                    for hh in range(2):
                        lhs = jnp.where(row16 == 2 * jj + hh, x16, 0.0).astype(_BF16)
                        acc = acc + _dot(lhs, ws[hh])
                        yield
                q_ref[gi] = acc
        return gen, 8 * len(gis)

    def qabs_piece(gi):
        def gen():
            qg = q_ref[gi]
            acc = jnp.zeros((16, _D), _F32)
            for jj in range(4):
                ws = head_pair(4 * gi + jj)
                for hh in range(2):
                    lhs = jnp.where(row16h == 2 * jj + hh, qg, 0.0).astype(_BF16)
                    acc = acc + _dot_nt(lhs, ws[hh])
                    yield
            qabs_ref[0, gi * 8:(gi + 1) * 8, :] = acc[0:8]
            qabs_ref[1, gi * 8:(gi + 1) * 8, :] = acc[8:16]
        return gen, 8

    def cblk(b, r0):
        half, r = r0 // (_SK // 2), r0 % (_SK // 2)
        return cbuf[b, half, r // r_ck, pl.ds(r % r_ck, _SUB), :]

    def scores_piece(b, i):
        def gen():
            if (i * _CH) % (_SK // 2) == 0:
                hf = i * _CH // (_SK // 2)
                wait_all(cbuf.at[b, hf], w_sem.at[6 + 2 * b + hf])
            qb = qabs_ref[b].astype(_BF16)
            mx = None if i == 0 else mx_ref[...]
            for u in range(_CH // _SUB):
                s = _dot_nt(qb, cblk(b, i * _CH + u * _SUB)) * scale
                s_ref[i, :, pl.ds(u * _SUB, _SUB)] = s
                for t in range(_SUB // 128):
                    st = s[:, t * 128:(t + 1) * 128]
                    mx = st if mx is None else jnp.maximum(mx, st)
                yield
            mx_ref[...] = mx
        return gen, _CH // _SUB

    def pv_piece(b, i):
        def gen():
            m = jnp.max(mx_ref[...], axis=1, keepdims=True)
            l = None if i == 0 else l_ref[...]
            acc = None if i == 0 else acc_ref[...]
            for u in range(_CH // _SUB):
                p = jnp.exp(s_ref[i, :, pl.ds(u * _SUB, _SUB)] - m)
                for t in range(_SUB // 128):
                    pt = p[:, t * 128:(t + 1) * 128]
                    l = pt if l is None else l + pt
                a = _dot(p.astype(_BF16), cblk(b, i * _CH + u * _SUB))
                acc = a if acc is None else acc + a
                yield
            if i == _SK // _CH - 1:
                ctx_ref[b] = acc / jnp.sum(l, axis=1, keepdims=True)
            else:
                l_ref[...] = l
                acc_ref[...] = acc
        return gen, _CH // _SUB

    def wo_rows(w, h):
        per = r_wo // _DH
        return w[h // per, pl.ds(pl.multiple_of((h % per) * _DH, _DH), _DH), :]

    def out_piece(gi):
        def gen():
            if gi == 0:
                wait_all(wob, w_sem.at[5])
            cg = jnp.concatenate([ctx_ref[0, gi * 8:(gi + 1) * 8, :],
                                  ctx_ref[1, gi * 8:(gi + 1) * 8, :]], axis=0)
            acc = jnp.zeros((16, _DH), _F32)
            for jj in range(4):
                ws = head_pair(4 * gi + jj)
                for hh in range(2):
                    lhs = jnp.where(row16 == 2 * jj + hh, cg, 0.0).astype(_BF16)
                    acc = acc + _dot(lhs, ws[hh])
                    yield
            out16 = jnp.zeros((16, _D), _F32)
            for r in range(8):
                lhs = jnp.where(row16h == r, acc, 0.0).astype(_BF16)
                out16 = out16 + _dot(lhs, wo_rows(wob, gi * 8 + r))
                yield
            s0 = jnp.sum(out16[0:8], axis=0, keepdims=True)
            s1 = jnp.sum(out16[8:16], axis=0, keepdims=True)
            part = jnp.where(row8 == 0, s0, jnp.where(row8 == 1, s1, 0.0))
            outb_ref[...] = part if gi == 0 else outb_ref[...] + part
        return gen, 16

    def attn_pieces(b):
        n = _SK // _CH
        return [scores_piece(b, i) for i in range(n)] + [pv_piece(b, i) for i in range(n)]

    stages = [
        ([to_u32(wqb, w_sem.at[2]), q_piece([0, 1]), q_piece([2, 3])], d_wuk),
        ([to_u32(wuk, w_sem.at[3])] + [qabs_piece(gi) for gi in range(4)], d_c[0] + d_c[1]),
        (attn_pieces(0), d_c[2] + d_c[3]),
        (attn_pieces(1), d_wuv + d_wob),
        ([to_u32(wuv, w_sem.at[4])] + [out_piece(gi) for gi in range(4)], []),
    ]
    pieces = {}
    for ps, carried in stages:
        for (gen, n), carry in zip(ps, _chunks(carried, len(ps))):
            pieces[_T0 + len(pieces)] = (gen, n, carry)
    assert max(pieces) < nst

    row8h = lax.broadcasted_iota(jnp.int32, (8, _DH), 0)
    pk = _SK // _NP

    def rows_of(buf, slot, i):
        r0 = i * pk
        return buf[slot, r0 // r_kv, pl.ds(r0 % r_kv, pk), :]

    def a_head(h, outa):
        q8 = qa_ref[h].astype(_BF16)
        on = []
        for b in range(_B):
            t = 2 * h + b
            slot = t % _NSTEP
            descs = kv_descs(t + _LA, (b + _LA) % 2)
            cut = _split(len(descs), 2 * _NP)
            more = t + _LA < nst
            if b == 0:
                issue(d_wqb, h == 0)
            wait_all(kbuf.at[slot], k_sem.at[slot])
            ss, mx = [], None
            for i in range(_NP):
                issue(descs[cut[i]:cut[i + 1]], more)
                s = _dot_nt(q8, rows_of(kbuf, slot, i)) * scale
                ss.append(s)
                for j in range(pk // 128):
                    sj = s[:, j * 128:(j + 1) * 128]
                    mx = sj if mx is None else jnp.maximum(mx, sj)
            m = jnp.max(mx, axis=1, keepdims=True)
            wait_all(vbuf.at[slot], v_sem.at[slot])
            l = o = None
            for i in range(_NP):
                issue(descs[cut[_NP + i]:cut[_NP + i + 1]], more)
                p = jnp.exp(ss[i] - m)
                for j in range(pk // 128):
                    pj = p[:, j * 128:(j + 1) * 128]
                    l = pj if l is None else l + pj
                oi = _dot(p.astype(_BF16), rows_of(vbuf, slot, i))
                o = oi if o is None else o + oi
            on.append(o / jnp.sum(l, axis=1, keepdims=True))
            for tp, (gen, n, carry) in pieces.items():
                if tp % 2 == b:
                    pl.when(h == tp // 2)(lambda gen=gen, n=n, carry=carry: run(gen(), n, carry))

        pl.when(h == 0)(lambda: wait_all(woa, w_sem.at[1]))
        lhs = jnp.where(row8h == 0, on[0], jnp.where(row8h == 1, on[1], 0.0)).astype(_BF16)
        return outa + _dot(lhs, wo_rows(woa, h))

    outa = lax.fori_loop(0, _H, a_head, jnp.zeros((8, _D), _F32))
    res = (g * outa + (1.0 - g) * outb_ref[...]).astype(_BF16)
    o_ref[...] = res[0:_B]


@jax.jit
def pallas_gated_mix__mha_block_cached__compressed_kv_cla__decode_kernel(
    A_x: jax.Array,
    A_k_cache: jax.Array,
    A_v_cache: jax.Array,
    A_wq: jax.Array,
    A_wo: jax.Array,
    B_x: jax.Array,
    B_c_kv: jax.Array,
    B_w_q: jax.Array,
    B_w_uk: jax.Array,
    B_w_uv: jax.Array,
    B_w_o: jax.Array,
    gate_w: jax.Array,
):
    del B_x
    hd = _H * _DH
    kv3 = (_KV[0], _SK // _KV[0], _DH)
    w33 = (_W3[0], _D * _H // _W3[0], _DH)
    wo3 = (_WO[0], hd // _WO[0], _D)
    ck3 = (_CK[0], _SK // 2 // _CK[0], _D)
    scratch = [
        pltpu.VMEM((_B, _D), _BF16),
        pltpu.VMEM((_D,), _BF16),
        pltpu.VMEM((_NSTEP,) + kv3, _BF16),
        pltpu.VMEM((_NSTEP,) + kv3, _BF16),
        pltpu.VMEM((_D, hd), _BF16),
        pltpu.VMEM(wo3, _BF16),
        pltpu.VMEM((_B, 2) + ck3, _BF16),
        pltpu.VMEM(w33, _BF16),
        pltpu.VMEM(w33, _BF16),
        pltpu.VMEM(w33, _BF16),
        pltpu.VMEM(wo3, _BF16),
        pltpu.VMEM((_D * _H // 2 + 16, _DH), jnp.uint32),
        pltpu.VMEM((_H, 8, _DH), _F32),
        pltpu.VMEM((4, 16, _DH), _F32),
        pltpu.VMEM((_B, _H, _D), _F32),
        pltpu.VMEM((_SK // _CH, _H, _CH), _F32),
        pltpu.VMEM((_H, 128), _F32),
        pltpu.VMEM((_H, 128), _F32),
        pltpu.VMEM((_H, _D), _F32),
        pltpu.VMEM((_B, _H, _D), _F32),
        pltpu.VMEM((8, _D), _F32),
        pltpu.SemaphoreType.DMA((_NSTEP,)),
        pltpu.SemaphoreType.DMA((_NSTEP,)),
        pltpu.SemaphoreType.DMA((12,)),
    ]
    out = pl.pallas_call(
        _kernel,
        out_shape=jax.ShapeDtypeStruct((_B, _D), _BF16),
        in_specs=[pl.BlockSpec(memory_space=pl.ANY)] * 11,
        out_specs=pl.BlockSpec(memory_space=pltpu.VMEM),
        scratch_shapes=scratch,
        compiler_params=pltpu.CompilerParams(vmem_limit_bytes=100 * 1024 * 1024),
    )(A_x.reshape(_B, _D), gate_w,
      A_k_cache.reshape((_B, _H * kv3[0]) + kv3[1:]),
      A_v_cache.reshape((_B, _H * kv3[0]) + kv3[1:]),
      A_wq, A_wo.reshape(wo3), B_c_kv.reshape((_B, 2) + ck3),
      B_w_q.reshape(w33), B_w_uk.reshape(w33), B_w_uv.reshape(w33), B_w_o.reshape(wo3))
    return out.reshape(_B, 1, _D)
```

```python
import jax
import jax.numpy as jnp
import numpy as np
from jax import lax
import jax.experimental.pallas as pl
import jax.experimental.pallas.tpu as pltpu

_B, _H, _SK, _DH, _D = 2, 32, 8192, 128, 512
_NT = (((1,), (1,)), ((), ()))
_F32 = jnp.float32
_BF16 = jnp.bfloat16
_HI16 = np.uint32(0xFFFF0000)

_LA = 2
_NSTEP = 4
_KV = (4, (32, 64, 32, 32))
_W3 = (4, (32, 64))
_WO = (2, (16, 32))
_NWO = 8
_CK = (2, (16, 32))
_WQA = (16, (1536, 1536, 1024))
_PRE = 64
_NP = 8
_T0 = 4
_CH = 2048
_SUB = 512


def _dot(a, b):
    return jnp.dot(a, b, preferred_element_type=_F32)


def _dot_nt(a, b):
    return lax.dot_general(a, b, _NT, preferred_element_type=_F32)


def _plan(total, sizes):
    out, o = [], 0
    while o < total:
        w = min(sizes[len(out) % len(sizes)], total - o)
        out.append((o, w, len(out) % 2))
        o += w
    return out


def _split(n, parts):
    return [(n * i) // parts for i in range(parts + 1)]


def _chunks(lst, parts):
    c = _split(len(lst), parts)
    return [lst[c[i]:c[i + 1]] for i in range(parts)]


def _kernel(x_hbm, gw_hbm, k_hbm, v_hbm, wqa_hbm, woa_hbm, c_hbm, wqb_hbm, wuk_hbm,
            wuv_hbm, wob_hbm, o_ref,
            x_ref, gw_ref, kbuf, vbuf, wqa, woa, cbuf, wqb, wuk, wuv, wob, u32,
            qa_ref, on_ref, q_ref, qabs_ref, s_ref, mx_ref, l_ref, acc_ref, ctx_ref,
            outb_ref, k_sem, v_sem, w_sem, o_sem):
    scale = _DH ** -0.5
    nst = _B * _H
    g_kv, r_kv = _KV[0], _SK // _KV[0]
    r_w3, r_wo, r_ck = _D * _H // _W3[0], _H * _DH // _WO[0], _SK // 2 // _CK[0]
    kv_plan, w3_plan = _plan(r_kv, _KV[1]), _plan(r_w3, _W3[1])
    wo_plan, ck_plan = _plan(r_wo, _WO[1]), _plan(r_ck, _CK[1])

    def descs3(src, dst, plan, sem):
        return [(src.at[:, pl.ds(o, w), :], dst.at[:, pl.ds(o, w), :], pr, sem)
                for (o, w, pr) in plan]

    def issue(descs, cond=None):
        def go():
            for (src, dst, pr, sem) in descs:
                pltpu.make_async_copy(src, dst, sem).start(priority=pr)
        if descs and cond is None:
            go()
        elif descs:
            pl.when(cond)(go)

    def wait_all(dst, sem):
        pltpu.make_async_copy(dst, dst, sem).wait()

    def run(gen, n, carry):
        cut = _split(len(carry), n)
        for i in range(n):
            issue(carry[cut[i]:cut[i + 1]])
            next(gen)
        for _ in gen:
            pass

    def kv_descs(t, b):
        h, slot = t // 2, t % _NSTEP
        hs = pl.ds(h * g_kv, g_kv)
        return (descs3(k_hbm.at[b, hs], kbuf.at[slot], kv_plan, k_sem.at[slot])
                + descs3(v_hbm.at[b, hs], vbuf.at[slot], kv_plan, v_sem.at[slot]))

    d_wqa = []
    for r0 in range(0, _D, _WQA[0]):
        c0 = 0
        for nc in _WQA[1]:
            idx = (pl.ds(r0, _WQA[0]), pl.ds(c0, nc))
            d_wqa.append((wqa_hbm.at[idx], wqa.at[idx], 0, w_sem.at[0]))
            c0 += nc
    r_part = r_wo // _NWO
    d_woa = [d for i in range(_NWO) for d in descs3(
        woa_hbm.at[:, pl.ds(i * r_part, r_part), :], woa.at[:, pl.ds(i * r_part, r_part), :],
        _plan(r_part, _WO[1]), o_sem.at[i])]
    d_wqb = descs3(wqb_hbm, wqb, w3_plan, w_sem.at[2])
    d_wuk = descs3(wuk_hbm, wuk, w3_plan, w_sem.at[3])
    d_wuv = descs3(wuv_hbm, wuv, w3_plan, w_sem.at[4])
    d_wob = descs3(wob_hbm, wob, wo_plan, w_sem.at[5])
    d_c = [descs3(c_hbm.at[b, hf], cbuf.at[b, hf], ck_plan, w_sem.at[6 + 2 * b + hf])
           for b in range(_B) for hf in range(2)]

    cp_x = pltpu.make_async_copy(x_hbm, x_ref, w_sem.at[10])
    cp_g = pltpu.make_async_copy(gw_hbm, gw_ref, w_sem.at[11])
    def with_prio(descs, pr):
        return [(src, dst, pr, sem) for (src, dst, _, sem) in descs]

    assert _LA == _B == 2
    kv01 = kv_descs(0, 0) + kv_descs(1, 1)
    cp_x.start()
    cp_g.start()
    issue(with_prio(kv01[:_PRE], 1))
    for i, d in enumerate(d_wqa):
        issue([d] + with_prio([kv01[_PRE + i]], 1))
    n_pre = _PRE + len(d_wqa)
    u32[pl.ds(_D * _H // 2, 16), :] = jnp.zeros((16, _DH), jnp.uint32)
    cp_x.wait()
    cp_g.wait()

    row8 = lax.broadcasted_iota(jnp.int32, (8, _D), 0)
    xf = x_ref[...].astype(_F32)
    x0 = jnp.broadcast_to(xf[0:1], (8, _D))
    x1 = jnp.broadcast_to(xf[1:2], (8, _D))
    x8 = jnp.where(row8 == 0, x0, jnp.where(row8 == 1, x1, 0.0))
    gw = gw_ref[...].reshape(1, _D).astype(_F32)
    g = jax.nn.sigmoid(jnp.sum(x8 * gw, axis=1, keepdims=True))

    def qa_gen():
        wait_all(wqa, w_sem.at[0])
        x8b = x8.astype(_BF16)
        for h in range(_H):
            qa_ref[h] = _dot(x8b, wqa[:, h * _DH:(h + 1) * _DH])
            yield
    run(qa_gen(), _H, kv01[n_pre:])

    row16 = lax.broadcasted_iota(jnp.int32, (16, _D), 0) % 8
    row16h = lax.broadcasted_iota(jnp.int32, (16, _DH), 0) % 8

    def to_u32(w, sem):
        def gen():
            wait_all(w, sem)
            n = r_w3 // 1024
            for i in range(16):
                v = w[i // n, pl.ds((i % n) * 1024, 1024), :]
                u32[pl.ds(i * 512, 512), :] = pltpu.bitcast(v, jnp.uint32)
                yield
        return gen, 16

    def head_pair(j):
        u = u32[pl.ds(j, _D, stride=16), :]
        lo = pltpu.bitcast(u << 16, _F32).astype(_BF16)
        hi = pltpu.bitcast(u & _HI16, _F32).astype(_BF16)
        return lo, hi

    def q_piece(gis):
        def gen():
            x16 = jnp.concatenate([x0, x1], axis=0)
            for gi in gis:
                acc = jnp.zeros((16, _DH), _F32)
                for jj in range(4):
                    ws = head_pair(4 * gi + jj)
                    for hh in range(2):
                        lhs = jnp.where(row16 == 2 * jj + hh, x16, 0.0).astype(_BF16)
                        acc = acc + _dot(lhs, ws[hh])
                        yield
                q_ref[gi] = acc
        return gen, 8 * len(gis)

    def qabs_piece(gi):
        def gen():
            qg = q_ref[gi]
            acc = jnp.zeros((16, _D), _F32)
            for jj in range(4):
                ws = head_pair(4 * gi + jj)
                for hh in range(2):
                    lhs = jnp.where(row16h == 2 * jj + hh, qg, 0.0).astype(_BF16)
                    acc = acc + _dot_nt(lhs, ws[hh])
                    yield
            qabs_ref[0, gi * 8:(gi + 1) * 8, :] = acc[0:8]
            qabs_ref[1, gi * 8:(gi + 1) * 8, :] = acc[8:16]
        return gen, 8

    def cblk(b, r0):
        half, r = r0 // (_SK // 2), r0 % (_SK // 2)
        return cbuf[b, half, r // r_ck, pl.ds(r % r_ck, _SUB), :]

    def scores_piece(b, i):
        def gen():
            if (i * _CH) % (_SK // 2) == 0:
                hf = i * _CH // (_SK // 2)
                wait_all(cbuf.at[b, hf], w_sem.at[6 + 2 * b + hf])
            qb = qabs_ref[b].astype(_BF16)
            mx = None if i == 0 else mx_ref[...]
            for u in range(_CH // _SUB):
                s = _dot_nt(qb, cblk(b, i * _CH + u * _SUB)) * scale
                s_ref[i, :, pl.ds(u * _SUB, _SUB)] = s
                for t in range(_SUB // 128):
                    st = s[:, t * 128:(t + 1) * 128]
                    mx = st if mx is None else jnp.maximum(mx, st)
                yield
            mx_ref[...] = mx
        return gen, _CH // _SUB

    def pv_piece(b, i):
        def gen():
            m = jnp.max(mx_ref[...], axis=1, keepdims=True)
            l = None if i == 0 else l_ref[...]
            acc = None if i == 0 else acc_ref[...]
            for u in range(_CH // _SUB):
                p = jnp.exp(s_ref[i, :, pl.ds(u * _SUB, _SUB)] - m)
                for t in range(_SUB // 128):
                    pt = p[:, t * 128:(t + 1) * 128]
                    l = pt if l is None else l + pt
                a = _dot(p.astype(_BF16), cblk(b, i * _CH + u * _SUB))
                acc = a if acc is None else acc + a
                yield
            if i == _SK // _CH - 1:
                ctx_ref[b] = acc / jnp.sum(l, axis=1, keepdims=True)
            else:
                l_ref[...] = l
                acc_ref[...] = acc
        return gen, _CH // _SUB

    def wo_rows(w, h):
        per = r_wo // _DH
        return w[h // per, pl.ds(pl.multiple_of((h % per) * _DH, _DH), _DH), :]

    def out_piece(gi):
        def gen():
            if gi == 0:
                wait_all(wob, w_sem.at[5])
            cg = jnp.concatenate([ctx_ref[0, gi * 8:(gi + 1) * 8, :],
                                  ctx_ref[1, gi * 8:(gi + 1) * 8, :]], axis=0)
            acc = jnp.zeros((16, _DH), _F32)
            for jj in range(4):
                ws = head_pair(4 * gi + jj)
                for hh in range(2):
                    lhs = jnp.where(row16 == 2 * jj + hh, cg, 0.0).astype(_BF16)
                    acc = acc + _dot(lhs, ws[hh])
                    yield
            out16 = jnp.zeros((16, _D), _F32)
            for r in range(8):
                lhs = jnp.where(row16h == r, acc, 0.0).astype(_BF16)
                out16 = out16 + _dot(lhs, wo_rows(wob, gi * 8 + r))
                yield
            s0 = jnp.sum(out16[0:8], axis=0, keepdims=True)
            s1 = jnp.sum(out16[8:16], axis=0, keepdims=True)
            part = jnp.where(row8 == 0, s0, jnp.where(row8 == 1, s1, 0.0))
            outb_ref[...] = part if gi == 0 else outb_ref[...] + part
        return gen, 16

    def attn_pieces(b):
        n = _SK // _CH
        return [scores_piece(b, i) for i in range(n)] + [pv_piece(b, i) for i in range(n)]

    stages = [
        ([to_u32(wqb, w_sem.at[2]), q_piece([0, 1]), q_piece([2, 3])], d_wuk),
        ([to_u32(wuk, w_sem.at[3])] + [qabs_piece(gi) for gi in range(4)], d_c[0] + d_c[1]),
        (attn_pieces(0), d_c[2] + d_c[3]),
        (attn_pieces(1), d_wuv + d_wob),
        ([to_u32(wuv, w_sem.at[4])] + [out_piece(gi) for gi in range(4)], []),
    ]
    pieces = {}
    for ps, carried in stages:
        for (gen, n), carry in zip(ps, _chunks(carried, len(ps))):
            pieces[_T0 + len(pieces)] = (gen, n, carry)
    assert max(pieces) < nst

    row8h = lax.broadcasted_iota(jnp.int32, (8, _DH), 0)
    pk = _SK // _NP

    def rows_of(buf, slot, i):
        r0 = i * pk
        return buf[slot, r0 // r_kv, pl.ds(r0 % r_kv, pk), :]

    def a_head(h, carry_):
        q8 = qa_ref[h].astype(_BF16)
        on = []
        for b in range(_B):
            t = 2 * h + b
            slot = t % _NSTEP
            descs = kv_descs(t + _LA, (b + _LA) % 2)
            cut = _split(len(descs), 2 * _NP)
            more = t + _LA < nst
            last = _chunks(_chunks(d_woa, _B)[b], 2 * _NP)
            fin = h == _H - 1

            def fetch(i, descs=descs, cut=cut, more=more, last=last, fin=fin):
                issue(descs[cut[i]:cut[i + 1]], more)
                issue(last[i], fin)
            if b == 0:
                issue(d_wqb, h == 0)
            wait_all(kbuf.at[slot], k_sem.at[slot])
            ss, mx = [], None
            for i in range(_NP):
                fetch(i)
                s = _dot_nt(q8, rows_of(kbuf, slot, i)) * scale
                ss.append(s)
                for j in range(pk // 128):
                    sj = s[:, j * 128:(j + 1) * 128]
                    mx = sj if mx is None else jnp.maximum(mx, sj)
            m = jnp.max(mx, axis=1, keepdims=True)
            wait_all(vbuf.at[slot], v_sem.at[slot])
            l = o = None
            for i in range(_NP):
                fetch(_NP + i)
                p = jnp.exp(ss[i] - m)
                for j in range(pk // 128):
                    pj = p[:, j * 128:(j + 1) * 128]
                    l = pj if l is None else l + pj
                oi = _dot(p.astype(_BF16), rows_of(vbuf, slot, i))
                o = oi if o is None else o + oi
            on.append(o / jnp.sum(l, axis=1, keepdims=True))
            for tp, (gen, n, carry) in pieces.items():
                if tp % 2 == b:
                    pl.when(h == tp // 2)(lambda gen=gen, n=n, carry=carry: run(gen(), n, carry))

        on_ref[h] = jnp.where(row8h == 0, on[0], jnp.where(row8h == 1, on[1], 0.0))
        return carry_

    lax.fori_loop(0, _H, a_head, 0)

    outa = jnp.zeros((8, _D), _F32)
    per = r_part // _DH
    for i in range(_NWO):
        wait_all(woa.at[:, pl.ds(i * r_part, r_part), :], o_sem.at[i])
        for gi in range(_WO[0]):
            for j in range(per):
                h = (gi * r_wo + i * r_part) // _DH + j
                outa = outa + _dot(on_ref[h].astype(_BF16),
                                   woa[gi, pl.ds(i * r_part + j * _DH, _DH), :])
    res = (g * outa + (1.0 - g) * outb_ref[...]).astype(_BF16)
    o_ref[...] = res[0:_B]


@jax.jit
def pallas_gated_mix__mha_block_cached__compressed_kv_cla__decode_kernel(
    A_x: jax.Array,
    A_k_cache: jax.Array,
    A_v_cache: jax.Array,
    A_wq: jax.Array,
    A_wo: jax.Array,
    B_x: jax.Array,
    B_c_kv: jax.Array,
    B_w_q: jax.Array,
    B_w_uk: jax.Array,
    B_w_uv: jax.Array,
    B_w_o: jax.Array,
    gate_w: jax.Array,
):
    del B_x
    hd = _H * _DH
    kv3 = (_KV[0], _SK // _KV[0], _DH)
    w33 = (_W3[0], _D * _H // _W3[0], _DH)
    wo3 = (_WO[0], hd // _WO[0], _D)
    ck3 = (_CK[0], _SK // 2 // _CK[0], _D)
    scratch = [
        pltpu.VMEM((_B, _D), _BF16),
        pltpu.VMEM((_D,), _BF16),
        pltpu.VMEM((_NSTEP,) + kv3, _BF16),
        pltpu.VMEM((_NSTEP,) + kv3, _BF16),
        pltpu.VMEM((_D, hd), _BF16),
        pltpu.VMEM(wo3, _BF16),
        pltpu.VMEM((_B, 2) + ck3, _BF16),
        pltpu.VMEM(w33, _BF16),
        pltpu.VMEM(w33, _BF16),
        pltpu.VMEM(w33, _BF16),
        pltpu.VMEM(wo3, _BF16),
        pltpu.VMEM((_D * _H // 2 + 16, _DH), jnp.uint32),
        pltpu.VMEM((_H, 8, _DH), _F32),
        pltpu.VMEM((_H, 8, _DH), _F32),
        pltpu.VMEM((4, 16, _DH), _F32),
        pltpu.VMEM((_B, _H, _D), _F32),
        pltpu.VMEM((_SK // _CH, _H, _CH), _F32),
        pltpu.VMEM((_H, 128), _F32),
        pltpu.VMEM((_H, 128), _F32),
        pltpu.VMEM((_H, _D), _F32),
        pltpu.VMEM((_B, _H, _D), _F32),
        pltpu.VMEM((8, _D), _F32),
        pltpu.SemaphoreType.DMA((_NSTEP,)),
        pltpu.SemaphoreType.DMA((_NSTEP,)),
        pltpu.SemaphoreType.DMA((12,)),
        pltpu.SemaphoreType.DMA((_NWO,)),
    ]
    out = pl.pallas_call(
        _kernel,
        out_shape=jax.ShapeDtypeStruct((_B, _D), _BF16),
        in_specs=[pl.BlockSpec(memory_space=pl.ANY)] * 11,
        out_specs=pl.BlockSpec(memory_space=pltpu.VMEM),
        scratch_shapes=scratch,
        compiler_params=pltpu.CompilerParams(vmem_limit_bytes=100 * 1024 * 1024),
    )(A_x.reshape(_B, _D), gate_w,
      A_k_cache.reshape((_B, _H * kv3[0]) + kv3[1:]),
      A_v_cache.reshape((_B, _H * kv3[0]) + kv3[1:]),
      A_wq, A_wo.reshape(wo3), B_c_kv.reshape((_B, 2) + ck3),
      B_w_q.reshape(w33), B_w_uk.reshape(w33), B_w_uv.reshape(w33), B_w_o.reshape(wo3))
    return out.reshape(_B, 1, _D)
```

```python
import jax
import jax.numpy as jnp
import numpy as np
from jax import lax
import jax.experimental.pallas as pl
import jax.experimental.pallas.tpu as pltpu

_B, _H, _SK, _DH, _D = 2, 32, 8192, 128, 512
_NT = (((1,), (1,)), ((), ()))
_F32 = jnp.float32
_BF16 = jnp.bfloat16
_HI16 = np.uint32(0xFFFF0000)

_LA = 2
_NSTEP = 4
_KV = (4, (32, 64, 32, 32))
_W3 = (4, (32, 64, 32, 32))
_WO = (4, (16, 8, 8, 8))
_CK = (4, (16, 8, 8, 8))
_WQA = (4, 8, (1024, 512, 512, 512, 1024, 512))
_NWO = 8
_PRE = 64
_NP = 8
_T0 = 4
_CH = 2048
_SUB = 512


def _dot(a, b):
    return jnp.dot(a, b, preferred_element_type=_F32)


def _dot_nt(a, b):
    return lax.dot_general(a, b, _NT, preferred_element_type=_F32)


def _plan(total, sizes):
    out, o = [], 0
    while o < total:
        w = min(sizes[len(out) % len(sizes)], total - o)
        out.append((o, w, len(out) % 2))
        o += w
    return out


def _split(n, parts):
    return [(n * i) // parts for i in range(parts + 1)]


def _chunks(lst, parts):
    c = _split(len(lst), parts)
    return [lst[c[i]:c[i + 1]] for i in range(parts)]


def _kernel(x_hbm, gw_hbm, k_hbm, v_hbm, wqa_hbm, woa_hbm, c_hbm, wqb_hbm, wuk_hbm,
            wuv_hbm, wob_hbm, o_ref,
            x_ref, gw_ref, kbuf, vbuf, wqa, woa, cbuf, wqb, wuk, wuv, wob, u32,
            qa_ref, on_ref, q_ref, qabs_ref, s_ref, mx_ref, l_ref, acc_ref, ctx_ref,
            outb_ref, k_sem, v_sem, w_sem, o_sem):
    scale = _DH ** -0.5
    nst = _B * _H
    g_kv, r_kv = _KV[0], _SK // _KV[0]
    r_w3, r_wo, r_ck = _D * _H // _W3[0], _H * _DH // _WO[0], _SK // 2 // _CK[0]
    kv_plan, w3_plan = _plan(r_kv, _KV[1]), _plan(r_w3, _W3[1])
    wo_plan, ck_plan = _plan(r_wo, _WO[1]), _plan(r_ck, _CK[1])

    def descs3(src, dst, plan, sem):
        return [(src.at[:, pl.ds(o, w), :], dst.at[:, pl.ds(o, w), :], pr, sem)
                for (o, w, pr) in plan]

    def issue(descs, cond=None):
        def go():
            for (src, dst, pr, sem) in descs:
                pltpu.make_async_copy(src, dst, sem).start(priority=pr)
        if descs and cond is None:
            go()
        elif descs:
            pl.when(cond)(go)

    def wait_all(dst, sem):
        pltpu.make_async_copy(dst, dst, sem).wait()

    def run(gen, n, carry):
        cut = _split(len(carry), n)
        for i in range(n):
            issue(carry[cut[i]:cut[i + 1]])
            next(gen)
        for _ in gen:
            pass

    def kv_descs(t, b):
        h, slot = t // 2, t % _NSTEP
        hs = pl.ds(h * g_kv, g_kv)
        return (descs3(k_hbm.at[b, hs], kbuf.at[slot], kv_plan, k_sem.at[slot])
                + descs3(v_hbm.at[b, hs], vbuf.at[slot], kv_plan, v_sem.at[slot]))

    d_wqa = []
    for r0 in range(0, _D // _WQA[0], _WQA[1]):
        c0 = 0
        for nc in _WQA[2]:
            idx = (slice(None), pl.ds(r0, _WQA[1]), pl.ds(c0, nc))
            d_wqa.append((wqa_hbm.at[idx], wqa.at[idx], 0, w_sem.at[0]))
            c0 += nc
    r_part = r_wo // _NWO
    assert r_part % _DH == 0
    d_woa = [d for i in range(_NWO) for d in descs3(
        woa_hbm.at[:, pl.ds(i * r_part, r_part), :], woa.at[:, pl.ds(i * r_part, r_part), :],
        _plan(r_part, _WO[1]), o_sem.at[i])]
    d_wqb = descs3(wqb_hbm, wqb, w3_plan, w_sem.at[2])
    d_wuk = descs3(wuk_hbm, wuk, w3_plan, w_sem.at[3])
    d_wuv = descs3(wuv_hbm, wuv, w3_plan, w_sem.at[4])
    d_wob = descs3(wob_hbm, wob, wo_plan, w_sem.at[5])
    d_c = [descs3(c_hbm.at[b, hf], cbuf.at[b, hf], ck_plan, w_sem.at[6 + 2 * b + hf])
           for b in range(_B) for hf in range(2)]

    cp_x = pltpu.make_async_copy(x_hbm, x_ref, w_sem.at[1])
    cp_g = pltpu.make_async_copy(gw_hbm, gw_ref, w_sem.at[10])

    def with_prio(descs, pr):
        return [(src, dst, pr, sem) for (src, dst, _, sem) in descs]

    assert _LA == _B == 2
    kv01 = kv_descs(0, 0) + kv_descs(1, 1)
    cp_x.start()
    cp_g.start()
    issue(with_prio(kv01[:_PRE], 1))
    for i, d in enumerate(d_wqa):
        issue([d] + with_prio([kv01[_PRE + i]], 1))
    n_pre = _PRE + len(d_wqa)
    u32[pl.ds(_D * _H // 2, 16), :] = jnp.zeros((16, _DH), jnp.uint32)
    cp_x.wait()
    cp_g.wait()

    row8 = lax.broadcasted_iota(jnp.int32, (8, _D), 0)
    xf = x_ref[...].astype(_F32)
    x0 = jnp.broadcast_to(xf[0:1], (8, _D))
    x1 = jnp.broadcast_to(xf[1:2], (8, _D))
    x8 = jnp.where(row8 == 0, x0, jnp.where(row8 == 1, x1, 0.0))
    gw = gw_ref[...].reshape(1, _D).astype(_F32)
    g = jax.nn.sigmoid(jnp.sum(x8 * gw, axis=1, keepdims=True))

    def qa_gen():
        wait_all(wqa, w_sem.at[0])
        x8b = x8.astype(_BF16)
        for h in range(_H):
            w = wqa[:, :, h * _DH:(h + 1) * _DH].reshape(_D, _DH)
            qa_ref[h] = _dot(x8b, w)
            yield
    run(qa_gen(), _H, kv01[n_pre:])

    row16 = lax.broadcasted_iota(jnp.int32, (16, _D), 0) % 8
    row16h = lax.broadcasted_iota(jnp.int32, (16, _DH), 0) % 8

    def to_u32(w, sem):
        def gen():
            wait_all(w, sem)
            n = r_w3 // 1024
            for i in range(16):
                v = w[i // n, pl.ds((i % n) * 1024, 1024), :]
                u32[pl.ds(i * 512, 512), :] = pltpu.bitcast(v, jnp.uint32)
                yield
        return gen, 16

    def head_pair(j):
        u = u32[pl.ds(j, _D, stride=16), :]
        lo = pltpu.bitcast(u << 16, _F32).astype(_BF16)
        hi = pltpu.bitcast(u & _HI16, _F32).astype(_BF16)
        return lo, hi

    def q_piece(gis):
        def gen():
            x16 = jnp.concatenate([x0, x1], axis=0)
            for gi in gis:
                acc = jnp.zeros((16, _DH), _F32)
                for jj in range(4):
                    ws = head_pair(4 * gi + jj)
                    for hh in range(2):
                        lhs = jnp.where(row16 == 2 * jj + hh, x16, 0.0).astype(_BF16)
                        acc = acc + _dot(lhs, ws[hh])
                        yield
                q_ref[gi] = acc
        return gen, 8 * len(gis)

    def qabs_piece(gi):
        def gen():
            qg = q_ref[gi]
            acc = jnp.zeros((16, _D), _F32)
            for jj in range(4):
                ws = head_pair(4 * gi + jj)
                for hh in range(2):
                    lhs = jnp.where(row16h == 2 * jj + hh, qg, 0.0).astype(_BF16)
                    acc = acc + _dot_nt(lhs, ws[hh])
                    yield
            qabs_ref[0, gi * 8:(gi + 1) * 8, :] = acc[0:8]
            qabs_ref[1, gi * 8:(gi + 1) * 8, :] = acc[8:16]
        return gen, 8

    def cblk(b, r0):
        half, r = r0 // (_SK // 2), r0 % (_SK // 2)
        return cbuf[b, half, r // r_ck, pl.ds(r % r_ck, _SUB), :]

    def scores_piece(b, i):
        def gen():
            if (i * _CH) % (_SK // 2) == 0:
                hf = i * _CH // (_SK // 2)
                wait_all(cbuf.at[b, hf], w_sem.at[6 + 2 * b + hf])
            qb = qabs_ref[b].astype(_BF16)
            mx = None if i == 0 else mx_ref[...]
            for u in range(_CH // _SUB):
                s = _dot_nt(qb, cblk(b, i * _CH + u * _SUB)) * scale
                s_ref[i, :, pl.ds(u * _SUB, _SUB)] = s
                for t in range(_SUB // 128):
                    st = s[:, t * 128:(t + 1) * 128]
                    mx = st if mx is None else jnp.maximum(mx, st)
                yield
            mx_ref[...] = mx
        return gen, _CH // _SUB

    def pv_piece(b, i):
        def gen():
            m = jnp.max(mx_ref[...], axis=1, keepdims=True)
            l = None if i == 0 else l_ref[...]
            acc = None if i == 0 else acc_ref[...]
            for u in range(_CH // _SUB):
                p = jnp.exp(s_ref[i, :, pl.ds(u * _SUB, _SUB)] - m)
                for t in range(_SUB // 128):
                    pt = p[:, t * 128:(t + 1) * 128]
                    l = pt if l is None else l + pt
                a = _dot(p.astype(_BF16), cblk(b, i * _CH + u * _SUB))
                acc = a if acc is None else acc + a
                yield
            if i == _SK // _CH - 1:
                ctx_ref[b] = acc / jnp.sum(l, axis=1, keepdims=True)
            else:
                l_ref[...] = l
                acc_ref[...] = acc
        return gen, _CH // _SUB

    def wo_rows(w, h):
        per = r_wo // _DH
        return w[h // per, pl.ds((h % per) * _DH, _DH), :]

    def out_piece(gi):
        def gen():
            if gi == 0:
                wait_all(wob, w_sem.at[5])
            cg = jnp.concatenate([ctx_ref[0, gi * 8:(gi + 1) * 8, :],
                                  ctx_ref[1, gi * 8:(gi + 1) * 8, :]], axis=0)
            acc = jnp.zeros((16, _DH), _F32)
            for jj in range(4):
                ws = head_pair(4 * gi + jj)
                for hh in range(2):
                    lhs = jnp.where(row16 == 2 * jj + hh, cg, 0.0).astype(_BF16)
                    acc = acc + _dot(lhs, ws[hh])
                    yield
            out16 = jnp.zeros((16, _D), _F32)
            for r in range(8):
                lhs = jnp.where(row16h == r, acc, 0.0).astype(_BF16)
                out16 = out16 + _dot(lhs, wo_rows(wob, gi * 8 + r))
                yield
            s0 = jnp.sum(out16[0:8], axis=0, keepdims=True)
            s1 = jnp.sum(out16[8:16], axis=0, keepdims=True)
            part = jnp.where(row8 == 0, s0, jnp.where(row8 == 1, s1, 0.0))
            outb_ref[...] = part if gi == 0 else outb_ref[...] + part
        return gen, 16

    def attn_pieces(b):
        n = _SK // _CH
        return [scores_piece(b, i) for i in range(n)] + [pv_piece(b, i) for i in range(n)]

    stages = [
        ([to_u32(wqb, w_sem.at[2]), q_piece([0, 1]), q_piece([2, 3])], d_wuk),
        ([to_u32(wuk, w_sem.at[3])] + [qabs_piece(gi) for gi in range(4)], d_c[0] + d_c[1]),
        (attn_pieces(0), d_c[2] + d_c[3]),
        (attn_pieces(1), d_wuv + d_wob),
        ([to_u32(wuv, w_sem.at[4])] + [out_piece(gi) for gi in range(4)], []),
    ]
    pieces = {}
    for ps, carried in stages:
        for (gen, n), carry in zip(ps, _chunks(carried, len(ps))):
            pieces[_T0 + len(pieces)] = (gen, n, carry)
    assert max(pieces) < nst

    row8h = lax.broadcasted_iota(jnp.int32, (8, _DH), 0)
    pk = _SK // _NP

    def rows_of(buf, slot, i):
        r0 = i * pk
        return buf[slot, r0 // r_kv, pl.ds(r0 % r_kv, pk), :]

    def a_head(h, carry_):
        q8 = qa_ref[h].astype(_BF16)
        on = []
        for b in range(_B):
            t = 2 * h + b
            slot = t % _NSTEP
            descs = kv_descs(jnp.minimum(t + _LA, nst - 1), (b + _LA) % 2)
            cut = _split(len(descs), 2 * _NP)
            more = t + _LA < nst
            last = _chunks(_chunks(d_woa, _B)[b], 2 * _NP)
            fin = h == _H - 1

            def fetch(i, descs=descs, cut=cut, more=more, last=last, fin=fin):
                issue(descs[cut[i]:cut[i + 1]], more)
                issue(last[i], fin)
            if b == 0:
                issue(d_wqb, h == 0)
            wait_all(kbuf.at[slot], k_sem.at[slot])
            ss, mx = [], None
            for i in range(_NP):
                fetch(i)
                s = _dot_nt(q8, rows_of(kbuf, slot, i)) * scale
                ss.append(s)
                for j in range(pk // 128):
                    sj = s[:, j * 128:(j + 1) * 128]
                    mx = sj if mx is None else jnp.maximum(mx, sj)
            m = jnp.max(mx, axis=1, keepdims=True)
            wait_all(vbuf.at[slot], v_sem.at[slot])
            l = o = None
            for i in range(_NP):
                fetch(_NP + i)
                p = jnp.exp(ss[i] - m)
                for j in range(pk // 128):
                    pj = p[:, j * 128:(j + 1) * 128]
                    l = pj if l is None else l + pj
                oi = _dot(p.astype(_BF16), rows_of(vbuf, slot, i))
                o = oi if o is None else o + oi
            on.append(o / jnp.sum(l, axis=1, keepdims=True))
            for tp, (gen, n, carry) in pieces.items():
                if tp % 2 == b:
                    pl.when(h == tp // 2)(lambda gen=gen, n=n, carry=carry: run(gen(), n, carry))

        on_ref[h] = jnp.where(row8h == 0, on[0], jnp.where(row8h == 1, on[1], 0.0))
        return carry_

    lax.fori_loop(0, _H, a_head, 0)

    outa = jnp.zeros((8, _D), _F32)
    per = r_part // _DH
    for i in range(_NWO):
        wait_all(woa.at[:, pl.ds(i * r_part, r_part), :], o_sem.at[i])
        for gi in range(_WO[0]):
            for j in range(per):
                h = (gi * r_wo + i * r_part) // _DH + j
                outa = outa + _dot(on_ref[h].astype(_BF16),
                                   woa[gi, pl.ds(i * r_part + j * _DH, _DH), :])
    res = (g * outa + (1.0 - g) * outb_ref[...]).astype(_BF16)
    o_ref[...] = res[0:_B]


@jax.jit
def pallas_gated_mix__mha_block_cached__compressed_kv_cla__decode_kernel(
    A_x: jax.Array,
    A_k_cache: jax.Array,
    A_v_cache: jax.Array,
    A_wq: jax.Array,
    A_wo: jax.Array,
    B_x: jax.Array,
    B_c_kv: jax.Array,
    B_w_q: jax.Array,
    B_w_uk: jax.Array,
    B_w_uv: jax.Array,
    B_w_o: jax.Array,
    gate_w: jax.Array,
):
    del B_x
    hd = _H * _DH
    kv3 = (_KV[0], _SK // _KV[0], _DH)
    w33 = (_W3[0], _D * _H // _W3[0], _DH)
    wq3 = (_WQA[0], _D // _WQA[0], hd)
    wo3 = (_WO[0], hd // _WO[0], _D)
    ck3 = (_CK[0], _SK // 2 // _CK[0], _D)
    scratch = [
        pltpu.VMEM((_B, _D), _BF16),
        pltpu.VMEM((_D,), _BF16),
        pltpu.VMEM((_NSTEP,) + kv3, _BF16),
        pltpu.VMEM((_NSTEP,) + kv3, _BF16),
        pltpu.VMEM(wq3, _BF16),
        pltpu.VMEM(wo3, _BF16),
        pltpu.VMEM((_B, 2) + ck3, _BF16),
        pltpu.VMEM(w33, _BF16),
        pltpu.VMEM(w33, _BF16),
        pltpu.VMEM(w33, _BF16),
        pltpu.VMEM(wo3, _BF16),
        pltpu.VMEM((_D * _H // 2 + 16, _DH), jnp.uint32),
        pltpu.VMEM((_H, 8, _DH), _F32),
        pltpu.VMEM((_H, 8, _DH), _F32),
        pltpu.VMEM((4, 16, _DH), _F32),
        pltpu.VMEM((_B, _H, _D), _F32),
        pltpu.VMEM((_SK // _CH, _H, _CH), _F32),
        pltpu.VMEM((_H, 128), _F32),
        pltpu.VMEM((_H, 128), _F32),
        pltpu.VMEM((_H, _D), _F32),
        pltpu.VMEM((_B, _H, _D), _F32),
        pltpu.VMEM((8, _D), _F32),
        pltpu.SemaphoreType.DMA((_NSTEP,)),
        pltpu.SemaphoreType.DMA((_NSTEP,)),
        pltpu.SemaphoreType.DMA((11,)),
        pltpu.SemaphoreType.DMA((_NWO,)),
    ]
    out = pl.pallas_call(
        _kernel,
        out_shape=jax.ShapeDtypeStruct((_B, _D), _BF16),
        in_specs=[pl.BlockSpec(memory_space=pl.ANY)] * 11,
        out_specs=pl.BlockSpec(memory_space=pltpu.VMEM),
        scratch_shapes=scratch,
        compiler_params=pltpu.CompilerParams(vmem_limit_bytes=96 * 1024 * 1024),
    )(A_x.reshape(_B, _D), gate_w,
      A_k_cache.reshape((_B, _H * kv3[0]) + kv3[1:]),
      A_v_cache.reshape((_B, _H * kv3[0]) + kv3[1:]),
      A_wq.reshape(wq3), A_wo.reshape(wo3), B_c_kv.reshape((_B, 2) + ck3),
      B_w_q.reshape(w33), B_w_uk.reshape(w33), B_w_uv.reshape(w33), B_w_o.reshape(wo3))
    return out.reshape(_B, 1, _D)
```
